```python
import os as _os
_os.environ.setdefault("JAX_PLATFORMS", "cpu")
import jax
import jax.numpy as jnp

def _softmax(x, axis=-1):
    return jax.nn.softmax(x, axis=axis)
def _gelu(x):
    return jax.nn.gelu(x, approximate=True)
def _silu(x):
    return jax.nn.silu(x)
def _sigmoid(x):
    return jax.nn.sigmoid(x)
def _layernorm(x, axis=-1, eps=1e-5):
    m = jnp.mean(x, axis=axis, keepdims=True)
    v = jnp.var(x, axis=axis, keepdims=True)
    return (x - m) / jnp.sqrt(v + eps)
def _scatter_add(tgt, idx, src, axis=0):
    return tgt.at[idx].add(src)
def _segment_sum(src, seg, n):
    return jax.ops.segment_sum(src, seg, n)
class _Rng:
    def __init__(self, key):
        self._k = key
    def _next(self):
        self._k, sub = jax.random.split(self._k)
        return sub
    def normal(self, shape):
        return jax.random.normal(self._next(), shape, dtype=jnp.bfloat16)
    def randint(self, lo, hi, shape):
        return jax.random.randint(self._next(), shape, lo, hi, dtype=jnp.int32)
    def uniform(self, shape, lo=0.0, hi=1.0):
        return jax.random.uniform(self._next(), shape, jnp.bfloat16, lo, hi)
    def permutation(self, n):
        return jax.random.permutation(self._next(), n)


kernel_name = 'concat_heads__mha_block_cached__mha_block_cached__near_ridge'

def setup_inputs():
    _rng = _Rng(jax.random.key(int.from_bytes(__import__("os").urandom(4), "little")))
    _w = (lambda a: (lambda t: t.astype(jnp.bfloat16) if jnp.issubdtype(t.dtype, jnp.floating) else t)(jnp.asarray(a)))
    def _A_setup():
        B, Sq, D = 8, 160, 512
        H, Sk, Dh = 32, 512, 128
        return {
            "x": _w((lambda *s: _rng.normal(s) * 0.8)(B, Sq, D)),
            "k_cache": _w((lambda *s: _rng.normal(s) * 0.8)(B, H, Sk, Dh)),
            "v_cache": _w((lambda *s: _rng.normal(s) * 0.05)(B, H, Sk, Dh)),
            "wq": _w((lambda *s: _rng.normal(s) * 0.8)(D, H * Dh) * (D ** -0.5)),
            "wo": _w((lambda *s: _rng.normal(s) * 0.05)(H * Dh, D) * ((H * Dh) ** -0.5)),
        }
    _A_in = _A_setup()

    def _B_setup():
        B, Sq, D = 8, 160, 512
        H, Sk, Dh = 32, 512, 128
        return {
            "x": _w((lambda *s: _rng.normal(s) * 0.8)(B, Sq, D)),
            "k_cache": _w((lambda *s: _rng.normal(s) * 0.8)(B, H, Sk, Dh)),
            "v_cache": _w((lambda *s: _rng.normal(s) * 0.05)(B, H, Sk, Dh)),
            "wq": _w((lambda *s: _rng.normal(s) * 0.8)(D, H * Dh) * (D ** -0.5)),
            "wo": _w((lambda *s: _rng.normal(s) * 0.05)(H * Dh, D) * ((H * Dh) ** -0.5)),
        }
    _B_in = _B_setup()

    return {
        "A_x": _A_in["x"],
        "A_k_cache": _A_in["k_cache"],
        "A_v_cache": _A_in["v_cache"],
        "A_wq": _A_in["wq"],
        "A_wo": _A_in["wo"],
        "B_x": _B_in["x"],
        "B_k_cache": _B_in["k_cache"],
        "B_v_cache": _B_in["v_cache"],
        "B_wq": _B_in["wq"],
        "B_wo": _B_in["wo"],
    }

def reference(A_x, A_k_cache, A_v_cache, A_wq, A_wo, B_x, B_k_cache, B_v_cache, B_wq, B_wo):
    def _A_ref(x, k_cache, v_cache, wq, wo):
        B, Sq, D = x.shape
        H, Dh = 32, 128
        q = (lambda x, *d: x.transpose(*d))((x @ wq).reshape(B, Sq, H, Dh), 0, 2, 1, 3)
        scores = jnp.einsum("bhqd,bhkd->bhqk", q, k_cache) * (Dh ** -0.5)
        p = _softmax(scores, axis=-1)
        o = jnp.einsum("bhqk,bhkd->bhqd", p, v_cache)
        return (lambda x, *d: x.transpose(*d))(o, 0, 2, 1, 3).reshape(B, Sq, H * Dh) @ wo

    def _B_ref(x, k_cache, v_cache, wq, wo):
        B, Sq, D = x.shape
        H, Dh = 32, 128
        q = (lambda x, *d: x.transpose(*d))((x @ wq).reshape(B, Sq, H, Dh), 0, 2, 1, 3)
        scores = jnp.einsum("bhqd,bhkd->bhqk", q, k_cache) * (Dh ** -0.5)
        p = _softmax(scores, axis=-1)
        o = jnp.einsum("bhqk,bhkd->bhqd", p, v_cache)
        return (lambda x, *d: x.transpose(*d))(o, 0, 2, 1, 3).reshape(B, Sq, H * Dh) @ wo

    a = _A_ref(A_x, A_k_cache, A_v_cache, A_wq, A_wo)
    b = _B_ref(B_x, B_k_cache, B_v_cache, B_wq, B_wo)
    return jnp.concatenate([a, b], axis=-1)
```

```python
import math

import jax
import jax.numpy as jnp
from jax import lax
import jax.experimental.pallas as pl
import jax.experimental.pallas.tpu as pltpu

B, SQ, D, H, SK, DH = 8, 160, 512, 32, 512, 128
M = B * SQ
G = 2
NG = H // G
W = G * DH
NBANK = 4
GG = 2
XPARTS = (2, 2, 2, 2)
Q0 = 512
QW = 896
NQL = (H * DH - Q0) // QW
assert Q0 + NQL * QW == H * DH and NQL == NBANK and sum(XPARTS) == B
XOFFS = tuple(sum(XPARTS[:i]) for i in range(len(XPARTS)))
NXP = len(XPARTS)
QSCALE = (DH ** -0.5) * math.log2(math.e)

_NT = (((1,), (1,)), ((), ()))


def _kernel(ax, ak, av, awq, awo, bx, bk, bv, bwq, bwo, o_hbm,
            xbuf, wqbuf, wobuf, qbuf, acc, obuf, kvbuf,
            xsem, wqsem, wosem, kvsem, osem):
    x_h, k_h, v_h, wq_h, wo_h = (ax, bx), (ak, bk), (av, bv), (awq, bwq), (awo, bwo)

    def x_copy(s, p):
        rows = pl.ds(XOFFS[p], XPARTS[p])
        return pltpu.make_async_copy(x_h[s].at[rows], xbuf.at[s, rows], xsem.at[s * NXP + p])

    def wq_copy0(s):
        cols = pl.ds(0, Q0)
        return pltpu.make_async_copy(wq_h[s].at[:, cols], wqbuf.at[s, :, cols], wqsem.at[s * (NQL + 1)])

    def wq_copy(s, i):
        cols = pl.ds(pl.multiple_of(Q0 + i * QW, 128), QW)
        return pltpu.make_async_copy(wq_h[s].at[:, cols], wqbuf.at[s, :, cols], wqsem.at[s * (NQL + 1) + 1 + i])

    def wo_start(g):
        for s in range(2):
            pltpu.make_async_copy(wo_h[s].at[pl.ds(pl.multiple_of(g * W, W), W)], wobuf.at[g, s], wosem.at[g]).start()

    def kv_start(g, b):
        bank = lax.rem(g, NBANK)
        for s in range(2):
            for t, src in enumerate((k_h[s], v_h[s])):
                pltpu.make_async_copy(src.bitcast(jnp.uint32).at[b, pl.ds(g * G, G)],
                                      kvbuf.at[bank, b, 2 * s + t], kvsem.at[bank]).start()

    def unit_start(g, b):
        if b == 0:
            wo_start(g)
        kv_start(g, b)

    def group_wait(g):
        bank = lax.rem(g, NBANK)
        pltpu.make_async_copy(wobuf.at[g], wobuf.at[g], wosem.at[g]).wait()
        pltpu.make_async_copy(kvbuf.at[bank], kvbuf.at[bank], kvsem.at[bank]).wait()

    def o_copy(b, s):
        cols = pl.ds(s * D, D)
        return pltpu.make_async_copy(obuf.at[b, :, cols], o_hbm.at[b, :, cols], osem.at[2 * b + s])

    wq_copy0(0).start()
    first = [x_copy(0, p) for p in range(NXP)] + [wq_copy0(1)] + [x_copy(1, p) for p in range(NXP)]

    def issue_first(i, c):
        for k, cp in enumerate(first):
            pl.when(i == k)(cp.start)
        return c
    lax.fori_loop(0, len(first), issue_first, 0)

    def issue_wq(i, c):
        wq_copy(0, i).start()
        wq_copy(1, i).start()
        return c
    lax.fori_loop(0, NQL, issue_wq, 0)
    acc[...] = jnp.zeros(acc.shape, acc.dtype)

    def q_proj(s, col0, width, p=None):
        if p is None:
            x, rows = xbuf[s].reshape(M, D), slice(None)
        else:
            x = xbuf[s, XOFFS[p]:XOFFS[p] + XPARTS[p]].reshape(XPARTS[p] * SQ, D)
            rows = pl.ds(XOFFS[p] * SQ // 2, XPARTS[p] * SQ // 2)
        o = 0
        while o < width:
            w = min(512, width - o)
            cols = pl.ds(col0 + o if isinstance(col0, int) else pl.multiple_of(col0 + o, 128), w)
            q = jnp.dot(x, wqbuf[s, :, cols], preferred_element_type=jnp.float32) * QSCALE
            qbuf[s, rows, cols] = pltpu.bitcast(q.astype(jnp.bfloat16), jnp.uint32)
            o += w

    wq_copy0(0).wait()
    for p in range(NXP):
        x_copy(0, p).wait()
        q_proj(0, 0, Q0, p)
    wq_copy0(1).wait()
    for p in range(NXP):
        x_copy(1, p).wait()
    q_proj(1, 0, Q0)

    def q_loop(i, c):
        wq_copy(0, i).wait()
        wq_copy(1, i).wait()
        for b in range(B):
            unit_start(i, b)
        for s in range(2):
            q_proj(s, Q0 + i * QW, QW)
        return c
    lax.fori_loop(0, NQL, q_loop, 0)

    def ao_loop(it, c):
        for gi in range(GG):
            g = it * GG + gi
            bank = lax.rem(g, NBANK)
            group_wait(g)
            for j in range(B):
                for s in range(2):
                    sc = []
                    for h in range(G):
                        col = pl.multiple_of((g * G + h) * DH, DH)
                        q = pltpu.bitcast(qbuf[s, pl.ds(j * SQ // 2, SQ // 2), pl.ds(col, DH)], jnp.bfloat16)
                        k = pltpu.bitcast(kvbuf[bank, j, 2 * s, h], jnp.bfloat16)
                        sc.append(lax.dot_general(q, k, _NT, preferred_element_type=jnp.float32))
                    pr = []
                    for h in range(G):
                        m = jnp.max(sc[h], axis=-1, keepdims=True)
                        e = jnp.exp2(sc[h] - m)
                        l = jnp.sum(e, axis=-1, keepdims=True)
                        pr.append((e.astype(jnp.bfloat16), 1.0 / l))
                    ov = []
                    for h in range(G):
                        v = pltpu.bitcast(kvbuf[bank, j, 2 * s + 1, h], jnp.bfloat16)
                        ov.append(jnp.dot(pr[h][0], v, preferred_element_type=jnp.float32) * pr[h][1])
                    if s == 1:
                        pl.when(g + NBANK < NG)(lambda: unit_start(g + NBANK, j))
                    r = None
                    for h in range(G):
                        rh = jnp.dot(ov[h].astype(jnp.bfloat16), wobuf[g, s, h * DH:(h + 1) * DH, :],
                                     preferred_element_type=jnp.float32)
                        r = rh if r is None else r + rh
                    new = acc[j, :, s * D:(s + 1) * D] + r
                    acc[j, :, s * D:(s + 1) * D] = new
                    if gi == GG - 1:
                        obuf[j, :, s * D:(s + 1) * D] = new.astype(jnp.bfloat16)
                        pl.when(g == NG - 1)(lambda: o_copy(j, s).start())
        return c
    lax.fori_loop(0, NG // GG, ao_loop, 0)

    for b in range(B):
        for s in range(2):
            o_copy(b, s).wait()


@jax.jit
def pallas_concat_heads__mha_block_cached__mha_block_cached__near_ridge_kernel(
    A_x: jax.Array,
    A_k_cache: jax.Array,
    A_v_cache: jax.Array,
    A_wq: jax.Array,
    A_wo: jax.Array,
    B_x: jax.Array,
    B_k_cache: jax.Array,
    B_v_cache: jax.Array,
    B_wq: jax.Array,
    B_wo: jax.Array,
):
    hbm = pl.BlockSpec(memory_space=pl.ANY)
    return pl.pallas_call(
        _kernel,
        in_specs=[hbm] * 10,
        out_specs=hbm,
        out_shape=jax.ShapeDtypeStruct((B, SQ, 2 * D), jnp.bfloat16),
        scratch_shapes=[
            pltpu.VMEM((2, B, SQ, D), jnp.bfloat16),
            pltpu.VMEM((2, D, H * DH), jnp.bfloat16),
            pltpu.VMEM((NG, 2, W, D), jnp.bfloat16),
            pltpu.VMEM((2, M // 2, H * DH), jnp.uint32),
            pltpu.VMEM((B, SQ, 2 * D), jnp.float32),
            pltpu.VMEM((B, SQ, 2 * D), jnp.bfloat16),
            pltpu.VMEM((NBANK, B, 4, G, SK // 2, DH), jnp.uint32),
            pltpu.SemaphoreType.DMA((2 * NXP,)),
            pltpu.SemaphoreType.DMA((2 * (NQL + 1),)),
            pltpu.SemaphoreType.DMA((NG,)),
            pltpu.SemaphoreType.DMA((NBANK,)),
            pltpu.SemaphoreType.DMA((2 * B,)),
        ],
        compiler_params=pltpu.CompilerParams(
            vmem_limit_bytes=100 * 1024 * 1024,
            disable_bounds_checks=True,
            flags={"XLA_TPU_RESCHEDULE_DMA_DONES": True},
        ),
    )(A_x, A_k_cache, A_v_cache, A_wq, A_wo, B_x, B_k_cache, B_v_cache, B_wq, B_wo)
```

```python
import math

import jax
import jax.numpy as jnp
from jax import lax
import jax.experimental.pallas as pl
import jax.experimental.pallas.tpu as pltpu

B, SQ, D, H, SK, DH = 8, 160, 512, 32, 512, 128
M = B * SQ
G = 2
NG = H // G
W = G * DH
NBANK = 4
GG = 2
SPIECES = ((0, 256), (256, 256), (512, 512))
SA = 1024
NQL = NBANK
QWA = (H * DH - SA) // NQL
QWB = H * DH // NQL
assert SA + NQL * QWA == H * DH and QWA % 128 == 0 and QWB % 128 == 0
QSCALE = (DH ** -0.5) * math.log2(math.e)

_NT = (((1,), (1,)), ((), ()))


def _kernel(ax, ak, av, awq, awo, bx, bk, bv, bwq, bwo, o_hbm,
            xbuf, wqbuf, wobuf, qbuf, acc, obuf, kvbuf,
            xsem, wqsem, wosem, kvsem, osem):
    x_h, k_h, v_h, wq_h, wo_h = (ax, bx), (ak, bk), (av, bv), (awq, bwq), (awo, bwo)

    def xa_copy(b):
        return pltpu.make_async_copy(x_h[0].at[b], xbuf.at[0, b], xsem.at[b])

    def xb_copy():
        return pltpu.make_async_copy(x_h[1], xbuf.at[1], xsem.at[B])

    def wq_piece(k):
        cols = pl.ds(*SPIECES[k])
        return pltpu.make_async_copy(wq_h[0].at[:, cols], wqbuf.at[0, :, cols], wqsem.at[k])

    def wq_chunk(s, i):
        col0, width = (SA + i * QWA, QWA) if s == 0 else (i * QWB, QWB)
        cols = pl.ds(pl.multiple_of(col0, 128), width)
        return pltpu.make_async_copy(wq_h[s].at[:, cols], wqbuf.at[s, :, cols],
                                     wqsem.at[len(SPIECES) + 2 * i + s])

    def wo_start(g):
        for s in range(2):
            pltpu.make_async_copy(wo_h[s].at[pl.ds(pl.multiple_of(g * W, W), W)], wobuf.at[g, s], wosem.at[g]).start()

    def kv_start(g, b):
        bank = lax.rem(g, NBANK)
        for s in range(2):
            for t, src in enumerate((k_h[s], v_h[s])):
                pltpu.make_async_copy(src.bitcast(jnp.uint32).at[b, pl.ds(g * G, G)],
                                      kvbuf.at[bank, b, 2 * s + t], kvsem.at[bank]).start()

    def unit_start(g, b):
        if b == 0:
            wo_start(g)
        kv_start(g, b)

    def group_wait(g):
        bank = lax.rem(g, NBANK)
        pltpu.make_async_copy(wobuf.at[g], wobuf.at[g], wosem.at[g]).wait()
        pltpu.make_async_copy(kvbuf.at[bank], kvbuf.at[bank], kvsem.at[bank]).wait()

    def o_copy(b, s):
        cols = pl.ds(s * D, D)
        return pltpu.make_async_copy(obuf.at[b, :, cols], o_hbm.at[b, :, cols], osem.at[2 * b + s])

    first = [wq_piece(0), xa_copy(0), wq_piece(1)] + [xa_copy(b) for b in range(1, B)] + [wq_piece(2), xb_copy()]
    first[0].start()

    def issue_first(i, c):
        for k, cp in enumerate(first[1:]):
            pl.when(i == k)(cp.start)
        return c
    lax.fori_loop(0, len(first) - 1, issue_first, 0)

    def issue_wq(i, c):
        wq_chunk(0, i).start()
        wq_chunk(1, i).start()
        return c
    lax.fori_loop(0, NQL, issue_wq, 0)

    def q_proj(s, col0, width, b=None):
        if b is None:
            x, rows = xbuf[s].reshape(M, D), slice(None)
        else:
            x, rows = xbuf[s, b], pl.ds(b * SQ // 2, SQ // 2)
        o = 0
        while o < width:
            w = min(512, width - o)
            cols = pl.ds(col0 + o if isinstance(col0, int) else pl.multiple_of(col0 + o, 128), w)
            q = jnp.dot(x, wqbuf[s, :, cols], preferred_element_type=jnp.float32) * QSCALE
            qbuf[s, rows, cols] = pltpu.bitcast(q.astype(jnp.bfloat16), jnp.uint32)
            o += w

    xa_copy(0).wait()
    for k in range(2):
        wq_piece(k).wait()
        q_proj(0, SPIECES[k][0], SPIECES[k][1], 0)
    for b in range(1, B):
        xa_copy(b).wait()
        q_proj(0, 0, 512, b)
    wq_piece(2).wait()
    q_proj(0, *SPIECES[2])
    xb_copy().wait()

    def q_loop(i, c):
        wq_chunk(0, i).wait()
        wq_chunk(1, i).wait()
        for b in range(B):
            unit_start(i, b)
        acc[pl.ds(i * (B // NQL), B // NQL)] = jnp.zeros((B // NQL, SQ, 2 * D), acc.dtype)
        q_proj(0, SA + i * QWA, QWA)
        q_proj(1, i * QWB, QWB)
        return c
    lax.fori_loop(0, NQL, q_loop, 0)

    def ao_loop(it, c):
        for gi in range(GG):
            g = it * GG + gi
            bank = lax.rem(g, NBANK)
            group_wait(g)
            for j in range(B):
                for s in range(2):
                    sc = []
                    for h in range(G):
                        col = pl.multiple_of((g * G + h) * DH, DH)
                        q = pltpu.bitcast(qbuf[s, pl.ds(j * SQ // 2, SQ // 2), pl.ds(col, DH)], jnp.bfloat16)
                        k = pltpu.bitcast(kvbuf[bank, j, 2 * s, h], jnp.bfloat16)
                        sc.append(lax.dot_general(q, k, _NT, preferred_element_type=jnp.float32))
                    pr = []
                    for h in range(G):
                        m = jnp.max(sc[h], axis=-1, keepdims=True)
                        e = jnp.exp2(sc[h] - m)
                        l = jnp.sum(e, axis=-1, keepdims=True)
                        pr.append((e.astype(jnp.bfloat16), 1.0 / l))
                    ov = []
                    for h in range(G):
                        v = pltpu.bitcast(kvbuf[bank, j, 2 * s + 1, h], jnp.bfloat16)
                        ov.append(jnp.dot(pr[h][0], v, preferred_element_type=jnp.float32) * pr[h][1])
                    if s == 1:
                        pl.when(g + NBANK < NG)(lambda: unit_start(g + NBANK, j))
                    r = None
                    for h in range(G):
                        rh = jnp.dot(ov[h].astype(jnp.bfloat16), wobuf[g, s, h * DH:(h + 1) * DH, :],
                                     preferred_element_type=jnp.float32)
                        r = rh if r is None else r + rh
                    new = acc[j, :, s * D:(s + 1) * D] + r
                    acc[j, :, s * D:(s + 1) * D] = new
                    if gi == GG - 1:
                        obuf[j, :, s * D:(s + 1) * D] = new.astype(jnp.bfloat16)
                        pl.when(g == NG - 1)(lambda: o_copy(j, s).start())
        return c
    lax.fori_loop(0, NG // GG, ao_loop, 0)

    for b in range(B):
        for s in range(2):
            o_copy(b, s).wait()


@jax.jit
def pallas_concat_heads__mha_block_cached__mha_block_cached__near_ridge_kernel(
    A_x: jax.Array,
    A_k_cache: jax.Array,
    A_v_cache: jax.Array,
    A_wq: jax.Array,
    A_wo: jax.Array,
    B_x: jax.Array,
    B_k_cache: jax.Array,
    B_v_cache: jax.Array,
    B_wq: jax.Array,
    B_wo: jax.Array,
):
    hbm = pl.BlockSpec(memory_space=pl.ANY)
    return pl.pallas_call(
        _kernel,
        in_specs=[hbm] * 10,
        out_specs=hbm,
        out_shape=jax.ShapeDtypeStruct((B, SQ, 2 * D), jnp.bfloat16),
        scratch_shapes=[
            pltpu.VMEM((2, B, SQ, D), jnp.bfloat16),
            pltpu.VMEM((2, D, H * DH), jnp.bfloat16),
            pltpu.VMEM((NG, 2, W, D), jnp.bfloat16),
            pltpu.VMEM((2, M // 2, H * DH), jnp.uint32),
            pltpu.VMEM((B, SQ, 2 * D), jnp.float32),
            pltpu.VMEM((B, SQ, 2 * D), jnp.bfloat16),
            pltpu.VMEM((NBANK, B, 4, G, SK // 2, DH), jnp.uint32),
            pltpu.SemaphoreType.DMA((B + 1,)),
            pltpu.SemaphoreType.DMA((len(SPIECES) + 2 * NQL,)),
            pltpu.SemaphoreType.DMA((NG,)),
            pltpu.SemaphoreType.DMA((NBANK,)),
            pltpu.SemaphoreType.DMA((2 * B,)),
        ],
        compiler_params=pltpu.CompilerParams(
            vmem_limit_bytes=100 * 1024 * 1024,
            disable_bounds_checks=True,
            disable_semaphore_checks=True,
            flags={"XLA_TPU_RESCHEDULE_DMA_DONES": True},
        ),
    )(A_x, A_k_cache, A_v_cache, A_wq, A_wo, B_x, B_k_cache, B_v_cache, B_wq, B_wo)
```

```python
import math

import jax
import jax.numpy as jnp
from jax import lax
import jax.experimental.pallas as pl
import jax.experimental.pallas.tpu as pltpu

B, SQ, D, H, SK, DH = 8, 160, 512, 32, 512, 128
M = B * SQ
G = 2
NG = H // G
W = G * DH
NBANK = 4
GG = 2
SPIECES = ((0, 256), (256, 256), (512, 512))
SA = 1024
NQL = NBANK
QWA = (H * DH - SA) // NQL
QWB = H * DH // NQL
assert SA + NQL * QWA == H * DH and QWA % 128 == 0 and QWB % 128 == 0
QSCALE = (DH ** -0.5) * math.log2(math.e)

_NT = (((1,), (1,)), ((), ()))


def _kernel(ax, ak, av, awq, awo, bx, bk, bv, bwq, bwo, o_hbm,
            xbuf, wqbuf, wobuf, qbuf, acc, obuf, kvbuf,
            xsem, wqsem, wosem, kvsem, osem):
    x_h, k_h, v_h, wq_h, wo_h = (ax, bx), (ak, bk), (av, bv), (awq, bwq), (awo, bwo)

    def xa_copy(b):
        return pltpu.make_async_copy(x_h[0].at[b], xbuf.at[0, b], xsem.at[b])

    def xb_copy():
        return pltpu.make_async_copy(x_h[1], xbuf.at[1], xsem.at[B])

    def wq_piece(k):
        cols = pl.ds(*SPIECES[k])
        return pltpu.make_async_copy(wq_h[0].at[:, cols], wqbuf.at[0, :, cols], wqsem.at[k])

    def wq_chunk(s, i):
        col0, width = (SA + i * QWA, QWA) if s == 0 else (i * QWB, QWB)
        cols = pl.ds(pl.multiple_of(col0, 128), width)
        return pltpu.make_async_copy(wq_h[s].at[:, cols], wqbuf.at[s, :, cols],
                                     wqsem.at[len(SPIECES) + 2 * i + s])

    def wo_start(g):
        for s in range(2):
            pltpu.make_async_copy(wo_h[s].at[pl.ds(pl.multiple_of(g * W, W), W)], wobuf.at[g, s], wosem.at[g]).start()

    def kv_start(g, b):
        bank = lax.rem(g, NBANK)
        for s in range(2):
            for t, src in enumerate((k_h[s], v_h[s])):
                pltpu.make_async_copy(src.at[b, pl.ds(g * G, G)], kvbuf.at[bank, b, 2 * s + t], kvsem.at[bank]).start()

    def unit_start(g, b):
        if b == 0:
            wo_start(g)
        kv_start(g, b)

    def group_wait(g):
        bank = lax.rem(g, NBANK)
        pltpu.make_async_copy(wobuf.at[g], wobuf.at[g], wosem.at[g]).wait()
        pltpu.make_async_copy(kvbuf.at[bank], kvbuf.at[bank], kvsem.at[bank]).wait()

    def o_copy(b, s):
        cols = pl.ds(s * D, D)
        return pltpu.make_async_copy(obuf.at[b, :, cols], o_hbm.at[b, :, cols], osem.at[2 * b + s])

    first = [wq_piece(0), xa_copy(0), wq_piece(1)] + [xa_copy(b) for b in range(1, B)] + [wq_piece(2), xb_copy()]
    first[0].start()

    def issue_first(i, c):
        for k, cp in enumerate(first[1:]):
            pl.when(i == k)(cp.start)
        return c
    lax.fori_loop(0, len(first) - 1, issue_first, 0)

    def issue_wq(i, c):
        wq_chunk(0, i).start()
        wq_chunk(1, i).start()
        return c
    lax.fori_loop(0, NQL, issue_wq, 0)

    def q_proj(s, col0, width, b=None):
        if b is None:
            x, rows = xbuf[s].reshape(M, D), slice(None)
        else:
            x, rows = xbuf[s, b], pl.ds(b * SQ, SQ)
        o = 0
        while o < width:
            w = min(512, width - o)
            cols = pl.ds(col0 + o if isinstance(col0, int) else pl.multiple_of(col0 + o, 128), w)
            q = jnp.dot(x, wqbuf[s, :, cols], preferred_element_type=jnp.float32) * QSCALE
            qbuf[s, rows, cols] = q.astype(jnp.bfloat16)
            o += w

    xa_copy(0).wait()
    for k in range(2):
        wq_piece(k).wait()
        q_proj(0, SPIECES[k][0], SPIECES[k][1], 0)
    for b in range(1, B):
        xa_copy(b).wait()
        q_proj(0, 0, 512, b)
    wq_piece(2).wait()
    q_proj(0, *SPIECES[2])
    xb_copy().wait()

    def q_loop(i, c):
        wq_chunk(0, i).wait()
        wq_chunk(1, i).wait()
        for b in range(B):
            unit_start(i, b)
        acc[pl.ds(i * (B // NQL), B // NQL)] = jnp.zeros((B // NQL, SQ, 2 * D), acc.dtype)
        q_proj(0, SA + i * QWA, QWA)
        q_proj(1, i * QWB, QWB)
        return c
    lax.fori_loop(0, NQL, q_loop, 0)

    def ao_loop(it, c):
        pending = []

        def out_proj():
            gi, j, s, ov = pending.pop()
            g = it * GG + gi
            o = jnp.concatenate(ov, axis=-1).astype(jnp.bfloat16)
            r = jnp.dot(o, wobuf[g, s], preferred_element_type=jnp.float32)
            new = acc[j, :, s * D:(s + 1) * D] + r
            acc[j, :, s * D:(s + 1) * D] = new
            if gi == GG - 1:
                obuf[j, :, s * D:(s + 1) * D] = new.astype(jnp.bfloat16)
                pl.when(g == NG - 1)(lambda: o_copy(j, s).start())

        for gi in range(GG):
            g = it * GG + gi
            bank = lax.rem(g, NBANK)
            group_wait(g)
            for j in range(B):
                for s in range(2):
                    pr = []
                    for h in range(G):
                        col = pl.multiple_of((g * G + h) * DH, DH)
                        q = qbuf[s, pl.ds(j * SQ, SQ), pl.ds(col, DH)]
                        sc = lax.dot_general(q, kvbuf[bank, j, 2 * s, h], _NT, preferred_element_type=jnp.float32)
                        m = jnp.max(sc, axis=-1, keepdims=True)
                        e = jnp.exp2(sc - m)
                        l = jnp.sum(e, axis=-1, keepdims=True)
                        pr.append((e.astype(jnp.bfloat16), 1.0 / l))
                        if h == 0 and pending:
                            out_proj()
                    ov = []
                    for h in range(G):
                        o = jnp.dot(pr[h][0], kvbuf[bank, j, 2 * s + 1, h], preferred_element_type=jnp.float32)
                        ov.append(o * pr[h][1])
                    if s == 1:
                        pl.when(g + NBANK < NG)(lambda: unit_start(g + NBANK, j))
                    pending.append((gi, j, s, ov))
        out_proj()
        return c
    lax.fori_loop(0, NG // GG, ao_loop, 0)

    for b in range(B):
        for s in range(2):
            o_copy(b, s).wait()


@jax.jit
def pallas_concat_heads__mha_block_cached__mha_block_cached__near_ridge_kernel(
    A_x: jax.Array,
    A_k_cache: jax.Array,
    A_v_cache: jax.Array,
    A_wq: jax.Array,
    A_wo: jax.Array,
    B_x: jax.Array,
    B_k_cache: jax.Array,
    B_v_cache: jax.Array,
    B_wq: jax.Array,
    B_wo: jax.Array,
):
    hbm = pl.BlockSpec(memory_space=pl.ANY)
    return pl.pallas_call(
        _kernel,
        in_specs=[hbm] * 10,
        out_specs=hbm,
        out_shape=jax.ShapeDtypeStruct((B, SQ, 2 * D), jnp.bfloat16),
        scratch_shapes=[
            pltpu.VMEM((2, B, SQ, D), jnp.bfloat16),
            pltpu.VMEM((2, D, H * DH), jnp.bfloat16),
            pltpu.VMEM((NG, 2, W, D), jnp.bfloat16),
            pltpu.VMEM((2, M, H * DH), jnp.bfloat16),
            pltpu.VMEM((B, SQ, 2 * D), jnp.float32),
            pltpu.VMEM((B, SQ, 2 * D), jnp.bfloat16),
            pltpu.VMEM((NBANK, B, 4, G, SK, DH), jnp.bfloat16),
            pltpu.SemaphoreType.DMA((B + 1,)),
            pltpu.SemaphoreType.DMA((len(SPIECES) + 2 * NQL,)),
            pltpu.SemaphoreType.DMA((NG,)),
            pltpu.SemaphoreType.DMA((NBANK,)),
            pltpu.SemaphoreType.DMA((2 * B,)),
        ],
        compiler_params=pltpu.CompilerParams(
            vmem_limit_bytes=100 * 1024 * 1024,
            disable_bounds_checks=True,
            disable_semaphore_checks=True,
            flags={"XLA_TPU_RESCHEDULE_DMA_DONES": True},
        ),
    )(A_x, A_k_cache, A_v_cache, A_wq, A_wo, B_x, B_k_cache, B_v_cache, B_wq, B_wo)
```

```python
import math

import jax
import jax.numpy as jnp
from jax import lax
import jax.experimental.pallas as pl
import jax.experimental.pallas.tpu as pltpu

B, SQ, D, H, SK, DH = 8, 160, 512, 32, 512, 128
M = B * SQ
G = 2
NG = H // G
W = G * DH
NBANK = 4
GG = 2
SPIECES = ((0, 256), (256, 256), (512, 512))
SA = 1024
NQL = NBANK
QWA = (H * DH - SA) // NQL
QWB = H * DH // NQL
assert SA + NQL * QWA == H * DH and QWA % 128 == 0 and QWB % 128 == 0
QSCALE = (DH ** -0.5) * math.log2(math.e)

_NT = (((1,), (1,)), ((), ()))


def _kernel(ax, ak, av, awq, awo, bx, bk, bv, bwq, bwo, o_hbm,
            xbuf, wqbuf, wobuf, qbuf, acc, obuf, kvbuf,
            xsem, wqsem, wosem, kvsem, osem):
    x_h, k_h, v_h, wq_h, wo_h = (ax, bx), (ak, bk), (av, bv), (awq, bwq), (awo, bwo)

    def xa_copy(b):
        return pltpu.make_async_copy(x_h[0].at[b], xbuf.at[0, b], xsem.at[b])

    def xb_copy():
        return pltpu.make_async_copy(x_h[1], xbuf.at[1], xsem.at[B])

    def wq_piece(k):
        cols = pl.ds(*SPIECES[k])
        return pltpu.make_async_copy(wq_h[0].at[:, cols], wqbuf.at[0, :, cols], wqsem.at[k])

    def wq_chunk(s, i):
        col0, width = (SA + i * QWA, QWA) if s == 0 else (i * QWB, QWB)
        cols = pl.ds(pl.multiple_of(col0, 128), width)
        return pltpu.make_async_copy(wq_h[s].at[:, cols], wqbuf.at[s, :, cols],
                                     wqsem.at[len(SPIECES) + 2 * i + s])

    def wo_start(g):
        for s in range(2):
            pltpu.make_async_copy(wo_h[s].at[pl.ds(pl.multiple_of(g * W, W), W)], wobuf.at[g, s], wosem.at[g]).start()

    def kv_start(g, b):
        bank = lax.rem(g, NBANK)
        for s in range(2):
            for t, src in enumerate((k_h[s], v_h[s])):
                pltpu.make_async_copy(src.at[b, pl.ds(g * G, G)], kvbuf.at[bank, b, 2 * s + t], kvsem.at[bank]).start()

    def unit_start(g, b):
        if b == 0:
            wo_start(g)
        kv_start(g, b)

    def wo_wait(g):
        pltpu.make_async_copy(wobuf.at[g], wobuf.at[g], wosem.at[g]).wait()

    def kv_wait(g):
        bank = lax.rem(g, NBANK)
        pltpu.make_async_copy(kvbuf.at[bank], kvbuf.at[bank], kvsem.at[bank]).wait()

    def o_copy(b, s):
        cols = pl.ds(s * D, D)
        return pltpu.make_async_copy(obuf.at[b, :, cols], o_hbm.at[b, :, cols], osem.at[2 * b + s])

    first = [wq_piece(0), xa_copy(0), wq_piece(1)] + [xa_copy(b) for b in range(1, B)] + [wq_piece(2), xb_copy()]
    first[0].start()

    def issue_first(i, c):
        for k, cp in enumerate(first[1:]):
            pl.when(i == k)(cp.start)
        return c
    lax.fori_loop(0, len(first) - 1, issue_first, 0)

    def issue_wq(i, c):
        wq_chunk(0, i).start()
        wq_chunk(1, i).start()
        return c
    lax.fori_loop(0, NQL, issue_wq, 0)

    def q_proj(s, col0, width, b=None):
        if b is None:
            x, rows = xbuf[s].reshape(M, D), slice(None)
        else:
            x, rows = xbuf[s, b], pl.ds(b * SQ, SQ)
        o = 0
        while o < width:
            w = min(512, width - o)
            cols = pl.ds(col0 + o if isinstance(col0, int) else pl.multiple_of(col0 + o, 128), w)
            q = jnp.dot(x, wqbuf[s, :, cols], preferred_element_type=jnp.float32) * QSCALE
            qbuf[s, rows, cols] = q.astype(jnp.bfloat16)
            o += w

    xa_copy(0).wait()
    for k in range(2):
        wq_piece(k).wait()
        q_proj(0, SPIECES[k][0], SPIECES[k][1], 0)
    for b in range(1, B):
        xa_copy(b).wait()
        q_proj(0, 0, 512, b)
    wq_piece(2).wait()
    q_proj(0, *SPIECES[2])
    xb_copy().wait()

    def q_loop(i, c):
        wq_chunk(0, i).wait()
        wq_chunk(1, i).wait()
        for b in range(B):
            unit_start(i, b)
        acc[pl.ds(i * (B // NQL), B // NQL)] = jnp.zeros((B // NQL, SQ, 2 * D), acc.dtype)
        q_proj(0, SA + i * QWA, QWA)
        q_proj(1, i * QWB, QWB)
        return c
    lax.fori_loop(0, NQL, q_loop, 0)

    def ao_loop(it, c):
        g0 = it * GG
        st = {}

        def step(n):
            return n // (2 * B), (n % (2 * B)) // 2, n % 2

        def scores(n, h):
            gi, j, s = step(n)
            col = pl.multiple_of(((g0 + gi) * G + h) * DH, DH)
            q = qbuf[s, pl.ds(j * SQ, SQ), pl.ds(col, DH)]
            k = kvbuf[lax.rem(g0 + gi, NBANK), j, 2 * s, h]
            st["s", n, h] = lax.dot_general(q, k, _NT, preferred_element_type=jnp.float32)

        def softmax(n, h):
            sc = st.pop(("s", n, h))
            m = jnp.max(sc, axis=-1, keepdims=True)
            e = jnp.exp2(sc - m)
            l = jnp.sum(e, axis=-1, keepdims=True)
            st["p", n, h] = (e.astype(jnp.bfloat16), 1.0 / l)

        def pv(n, h):
            gi, j, s = step(n)
            e, r = st.pop(("p", n, h))
            v = kvbuf[lax.rem(g0 + gi, NBANK), j, 2 * s + 1, h]
            st["o", n, h] = jnp.dot(e, v, preferred_element_type=jnp.float32) * r
            if s == 1 and h == G - 1:
                pl.when(g0 + gi + NBANK < NG)(lambda: unit_start(g0 + gi + NBANK, j))

        def out_proj(n):
            gi, j, s = step(n)
            g = g0 + gi
            o = jnp.concatenate([st.pop(("o", n, h)) for h in range(G)], axis=-1).astype(jnp.bfloat16)
            r = jnp.dot(o, wobuf[g, s], preferred_element_type=jnp.float32)
            new = acc[j, :, s * D:(s + 1) * D] + r
            acc[j, :, s * D:(s + 1) * D] = new
            if gi == GG - 1:
                obuf[j, :, s * D:(s + 1) * D] = new.astype(jnp.bfloat16)
                pl.when(g0 + gi == NG - 1)(lambda: o_copy(j, s).start())

        nsteps = GG * B * 2
        for n in range(nsteps):
            gi = step(n)[0]
            if n % (2 * B) == 0:
                wo_wait(g0 + gi)
                kv_wait(g0 + gi)
            scores(n, 0)
            softmax(n, 0)
            if n > 0:
                out_proj(n - 1)
            scores(n, 1)
            softmax(n, 1)
            pv(n, 0)
            pv(n, 1)
        out_proj(nsteps - 1)
        return c
    lax.fori_loop(0, NG // GG, ao_loop, 0)

    for b in range(B):
        for s in range(2):
            o_copy(b, s).wait()


@jax.jit
def pallas_concat_heads__mha_block_cached__mha_block_cached__near_ridge_kernel(
    A_x: jax.Array,
    A_k_cache: jax.Array,
    A_v_cache: jax.Array,
    A_wq: jax.Array,
    A_wo: jax.Array,
    B_x: jax.Array,
    B_k_cache: jax.Array,
    B_v_cache: jax.Array,
    B_wq: jax.Array,
    B_wo: jax.Array,
):
    hbm = pl.BlockSpec(memory_space=pl.ANY)
    return pl.pallas_call(
        _kernel,
        in_specs=[hbm] * 10,
        out_specs=hbm,
        out_shape=jax.ShapeDtypeStruct((B, SQ, 2 * D), jnp.bfloat16),
        scratch_shapes=[
            pltpu.VMEM((2, B, SQ, D), jnp.bfloat16),
            pltpu.VMEM((2, D, H * DH), jnp.bfloat16),
            pltpu.VMEM((NG, 2, W, D), jnp.bfloat16),
            pltpu.VMEM((2, M, H * DH), jnp.bfloat16),
            pltpu.VMEM((B, SQ, 2 * D), jnp.float32),
            pltpu.VMEM((B, SQ, 2 * D), jnp.bfloat16),
            pltpu.VMEM((NBANK, B, 4, G, SK, DH), jnp.bfloat16),
            pltpu.SemaphoreType.DMA((B + 1,)),
            pltpu.SemaphoreType.DMA((len(SPIECES) + 2 * NQL,)),
            pltpu.SemaphoreType.DMA((NG,)),
            pltpu.SemaphoreType.DMA((NBANK,)),
            pltpu.SemaphoreType.DMA((2 * B,)),
        ],
        compiler_params=pltpu.CompilerParams(
            vmem_limit_bytes=100 * 1024 * 1024,
            disable_bounds_checks=True,
            disable_semaphore_checks=True,
            flags={"XLA_TPU_RESCHEDULE_DMA_DONES": True},
        ),
    )(A_x, A_k_cache, A_v_cache, A_wq, A_wo, B_x, B_k_cache, B_v_cache, B_wq, B_wo)
```
